```python
import jax
import jax.numpy as jnp

def _softmax(x, axis=-1):
    return jax.nn.softmax(x, axis=axis)
def _gelu(x):
    return jax.nn.gelu(x, approximate=True)
def _silu(x):
    return jax.nn.silu(x)
def _sigmoid(x):
    return jax.nn.sigmoid(x)
def _layernorm(x, axis=-1, eps=1e-5):
    m = jnp.mean(x, axis=axis, keepdims=True)
    v = jnp.var(x, axis=axis, keepdims=True)
    return (x - m) / jnp.sqrt(v + eps)
def _scatter_add(tgt, idx, src, axis=0):
    return tgt.at[idx].add(src)
def _segment_sum(src, seg, n):
    return jax.ops.segment_sum(src, seg, n)
class _Rng:
    def __init__(self, key):
        self._k = key
    def _next(self):
        self._k, sub = jax.random.split(self._k)
        return sub
    def normal(self, shape):
        return jax.random.normal(self._next(), shape, dtype=jnp.bfloat16)
    def randint(self, lo, hi, shape):
        return jax.random.randint(self._next(), shape, lo, hi, dtype=jnp.int32)
    def uniform(self, shape, lo=0.0, hi=1.0):
        return jax.random.uniform(self._next(), shape, jnp.bfloat16, lo, hi)
    def permutation(self, n):
        return jax.random.permutation(self._next(), n)


kernel_name = 'interleave_layers__sliding_block_cached__glu_gated_glu__decode'

def setup_inputs():
    _rng = _Rng(jax.random.key(int.from_bytes(__import__("os").urandom(4), "little")))
    _w = (lambda a: (lambda t: t.astype(jnp.bfloat16) if jnp.issubdtype(t.dtype, jnp.floating) else t)(jnp.asarray(a)))
    def _A_setup():
        B, Sq, D = 1, 1, 640
        Hq, Hkv, Sk, Dh = 32, 32, 32768, 192
        assert Hq % Hkv == 0, (Hq, Hkv)
        return {
            "x": _w((lambda *s: _rng.normal(s) * 0.05)(B, Sq, D)),
            "k_cache": _w((lambda *s: _rng.normal(s) * 0.05)(B, Hkv, Sk, Dh)),
            "v_cache": _w((lambda *s: _rng.normal(s) * 0.05)(B, Hkv, Sk, Dh)),
            "wq": _w((lambda *s: _rng.normal(s) * 0.05)(D, Hq * Dh) * (D ** -0.5)),
            "wo": _w((lambda *s: _rng.normal(s) * 0.05)(Hq * Dh, D) * ((Hq * Dh) ** -0.5)),
        }
    _A_in = _A_setup()

    def _B_setup():
        B, S, D, F = 1, 1, 640, 1536
        return {
            "x": _w((lambda *s: _rng.normal(s) * 0.05)(B, S, D)),
            "w_gate": _w((lambda *s: _rng.normal(s) * 0.05)(D, F)),
            "w_up": _w((lambda *s: _rng.normal(s) * 0.05)(D, F)),
            "w_down": _w((lambda *s: _rng.normal(s) * 0.05)(F, D)),
        }
    _B_in = _B_setup()

    return {
        "A_x": _A_in["x"],
        "A_k_cache": _A_in["k_cache"],
        "A_v_cache": _A_in["v_cache"],
        "A_wq": _A_in["wq"],
        "A_wo": _A_in["wo"],
        "B_x": _B_in["x"],
        "B_w_gate": _B_in["w_gate"],
        "B_w_up": _B_in["w_up"],
        "B_w_down": _B_in["w_down"],
    }

def reference(A_x, A_k_cache, A_v_cache, A_wq, A_wo, B_x, B_w_gate, B_w_up, B_w_down):
    def _A_ref(x, k_cache, v_cache, wq, wo):
        B, Sq, D = x.shape
        Hq, Dh = 32, 192
        Hkv, Sk = k_cache.shape[1], k_cache.shape[2]
        W = min(4096, max(256, Sk // 4))
        rep = Hq // Hkv
        q = (lambda x, *d: x.transpose(*d))((x @ wq).reshape(B, Sq, Hq, Dh), 0, 2, 1, 3)
        k = jnp.repeat(k_cache[:, :, Sk - W:, :], rep, axis=1)
        v = jnp.repeat(v_cache[:, :, Sk - W:, :], rep, axis=1)
        scores = jnp.einsum("bhqd,bhkd->bhqk", q, k) * (Dh ** -0.5)
        p = _softmax(scores, axis=-1)
        o = jnp.einsum("bhqk,bhkd->bhqd", p, v)
        return (lambda x, *d: x.transpose(*d))(o, 0, 2, 1, 3).reshape(B, Sq, Hq * Dh) @ wo

    def _B_ref(x, w_gate, w_up, w_down):
        g = jnp.einsum("bsd,df->bsf", x, w_gate)
        u = jnp.einsum("bsd,df->bsf", x, w_up)
        h = _sigmoid(g) * u
        return jnp.einsum("bsf,fd->bsd", h, w_down)

    x = A_x
    x = x + _A_ref(_layernorm(x, axis=-1), A_k_cache, A_v_cache, A_wq, A_wo)
    x = x + _B_ref(_layernorm(x, axis=-1), B_w_gate, B_w_up, B_w_down)
    x = x + _A_ref(_layernorm(x, axis=-1), A_k_cache, A_v_cache, A_wq, A_wo)
    x = x + _B_ref(_layernorm(x, axis=-1), B_w_gate, B_w_up, B_w_down)
    return x
```

```python
import jax
import jax.numpy as jnp
from jax import lax
from jax.experimental import pallas as pl
from jax.experimental.pallas import tpu as pltpu

D, H, DH, SK, FF = 640, 32, 192, 32768, 1536
W = min(4096, max(256, SK // 4))
G = 8
NG = H // G
GR = G * DH
BF, F32, U32 = jnp.bfloat16, jnp.float32, jnp.uint32
LOG2E = 1.4426950408889634


def _bf(w):
    return pltpu.bitcast(w, BF)


def _dot(a, b):
    return jnp.dot(a, b, preferred_element_type=F32)


def _ln(x):
    m = jnp.mean(x, axis=-1, keepdims=True)
    c = x - m
    v = jnp.mean(c * c, axis=-1, keepdims=True)
    return c / jnp.sqrt(v + 1e-5)


def _kernel(x_hbm, k_hbm, v_hbm, wq_hbm, wo_hbm, wg_hbm, wu_hbm, wd_hbm, o_ref,
            x_v, k_v, v_v, wq_v, wo_v, wg_v, wu_v, wd_v, q_v, kv_sem, w_sem):
    win = pl.ds(SK - W, W)
    kb, vb = k_v.bitcast(BF), v_v.bitcast(BF)

    def k_copy(g):
        return pltpu.make_async_copy(k_hbm.at[g, :, win], kb.at[g], kv_sem.at[0, g])

    def v_copy(g):
        return pltpu.make_async_copy(v_hbm.at[g, :, win], vb.at[g], kv_sem.at[1, g])

    x_copy = pltpu.make_async_copy(x_hbm, x_v, w_sem.at[0])
    w_copies = [
        pltpu.make_async_copy(src, dst.bitcast(BF), w_sem.at[i + 1])
        for i, (src, dst) in enumerate(
            [(wq_hbm, wq_v), (wo_hbm, wo_v), (wg_hbm, wg_v), (wu_hbm, wu_v), (wd_hbm, wd_v)])
    ]
    x_copy.start()
    w_copies[0].start()
    for g in range(NG):
        v_copy(g).start()
    for g in range(NG):
        k_copy(g).start()
    for c in w_copies[1:]:
        c.start()

    def xpose_group(g, carry):
        v_copy(g).wait()

        def xpose_rows(i, carry):
            r = pl.ds(pl.multiple_of(i * 64, 64), 64)
            for j in range(W // 128):
                c = pl.ds(j * 128, 128)
                v_v[g, r, c] = pltpu.bitcast(_bf(v_v[g, r, c]).T, U32)
            return carry
        return lax.fori_loop(0, GR // 128, xpose_rows, carry)
    lax.fori_loop(0, NG, xpose_group, 0)

    x_copy.wait()
    x0 = jnp.broadcast_to(x_v[...].astype(F32), (8, D))
    diag = (lax.broadcasted_iota(jnp.int32, (G, GR), 1) // DH
            == lax.broadcasted_iota(jnp.int32, (G, GR), 0))

    def layer(it, x):
        first = it == 0

        @pl.when(first)
        def _():
            w_copies[0].wait()
        xn = _ln(x).astype(BF)
        for g in range(NG):
            q = _dot(xn, _bf(wq_v[:, g * GR:(g + 1) * GR]))
            q_v[g] = jnp.where(diag, q, 0.0)

        @pl.when(first)
        def _():
            for g in range(NG):
                k_copy(g).wait()

        def attend(g, carry):
            s = _dot(q_v[g].astype(BF), _bf(k_v[g]))
            m = jnp.max(s, axis=-1, keepdims=True)
            p = jnp.exp2((s - m) * (DH ** -0.5 * LOG2E))
            l = jnp.sum(p, axis=-1, keepdims=True)
            pb = p.astype(BF)
            outs = []
            for i in range(GR // 128):
                vt = jnp.concatenate(
                    [_bf(v_v[g, i * 64:(i + 1) * 64, j * 128:(j + 1) * 128])
                     for j in range(W // 128)], axis=0)
                outs.append(_dot(pb, vt))
            o = jnp.concatenate(outs, axis=1)
            q_v[g] = jnp.where(diag, o / l, 0.0)
            return carry
        lax.fori_loop(0, NG, attend, 0)

        @pl.when(first)
        def _():
            w_copies[1].wait()
        o = jnp.concatenate([q_v[g] for g in range(NG)], axis=1).astype(BF)
        a = _dot(o, _bf(wo_v[...]))
        x = x + jnp.sum(a, axis=0, keepdims=True)

        @pl.when(first)
        def _():
            w_copies[2].wait()
            w_copies[3].wait()
        xn = _ln(x).astype(BF)
        gate = _dot(xn, _bf(wg_v[...]))
        up = _dot(xn, _bf(wu_v[...]))
        h = (jax.nn.sigmoid(gate) * up).astype(BF)

        @pl.when(first)
        def _():
            w_copies[4].wait()
        return x + _dot(h, _bf(wd_v[...]))

    x = lax.fori_loop(0, 2, layer, x0)
    o_ref[...] = x[0:1].astype(o_ref.dtype)


@jax.jit
def pallas_interleave_layers__sliding_block_cached__glu_gated_glu__decode_kernel(
        A_x, A_k_cache, A_v_cache, A_wq, A_wo, B_x, B_w_gate, B_w_up, B_w_down):
    del B_x
    kt = jnp.swapaxes(A_k_cache[0], 1, 2).reshape(NG, GR, SK)
    vt = jnp.swapaxes(A_v_cache[0], 1, 2).reshape(NG, GR, SK)
    hbm = pl.BlockSpec(memory_space=pl.ANY)
    out = pl.pallas_call(
        _kernel,
        out_shape=jax.ShapeDtypeStruct((1, D), A_x.dtype),
        in_specs=[hbm] * 8,
        out_specs=pl.BlockSpec(memory_space=pltpu.VMEM),
        scratch_shapes=[
            pltpu.VMEM((1, D), BF),
            pltpu.VMEM((NG, GR // 2, W), U32),
            pltpu.VMEM((NG, GR // 2, W), U32),
            pltpu.VMEM((D // 2, H * DH), U32),
            pltpu.VMEM((H * DH // 2, D), U32),
            pltpu.VMEM((D // 2, FF), U32),
            pltpu.VMEM((D // 2, FF), U32),
            pltpu.VMEM((FF // 2, D), U32),
            pltpu.VMEM((NG, G, GR), F32),
            pltpu.SemaphoreType.DMA((2, NG)),
            pltpu.SemaphoreType.DMA((6,)),
        ],
        compiler_params=pltpu.CompilerParams(vmem_limit_bytes=127 * 2**20),
        name="v1",
    )(A_x.reshape(1, D), kt, vt, A_wq, A_wo, B_w_gate, B_w_up, B_w_down)
    return out.reshape(1, 1, D)
```

```python
import functools
import jax
import jax.numpy as jnp
import numpy as np
from jax import lax
from jax.experimental import pallas as pl
from jax.experimental.pallas import tpu as pltpu

D, H, DH, SK, FF = 640, 32, 192, 32768, 1536
W = min(4096, max(256, SK // 4))
NT = W // 128
HH = 16
HM = 10
MT = HM * DH // 128
RG = DH // 16
PR = DH // 2
BF, F32, U32 = jnp.bfloat16, jnp.float32, jnp.uint32
LOG2E = 1.4426950408889634


def _bf(w):
    return pltpu.bitcast(w, BF)


def _pk(x):
    return pltpu.bitcast(x.astype(BF), U32)


def _unpack(w):
    return (pltpu.bitcast(w << 16, F32),
            pltpu.bitcast(w & np.uint32(0xFFFF0000), F32))


def _dot(a, b):
    return jnp.dot(a, b, preferred_element_type=F32)


def _ln(x):
    m = jnp.mean(x, axis=-1, keepdims=True)
    c = x - m
    v = jnp.mean(c * c, axis=-1, keepdims=True)
    return c / jnp.sqrt(v + 1e-5)


def _t(i, n=128):
    return slice(i * n, (i + 1) * n)


def _half(r):
    return slice(0, 8) if (r * 128) // DH < 8 else slice(8, 16)


def _kernel(x_hbm, k_hbm, v_hbm, wq_hbm, wo_hbm, wg_hbm, wu_hbm, wd_hbm, o_ref,
            x_v, k_v, v_v, wq_v, wo_v, wg_v, wu_v, wd_v,
            ql_v, qc_v, part_v, sv_v, pl_v, pv_v, rl_v, acc_v, ol_v, ap_v,
            k_sem, v_sem, w_sem, *, scopes=False):
    win = pl.ds(SK - W, W)
    kb, vb = k_v.bitcast(BF), v_v.bitcast(BF)
    CK = 4 * DH
    CV = 2 * DH
    NCK, NCV = HH * DH // CK, HH * DH // CV
    NWO = 4

    def scope(name):
        return jax.named_scope(name)

    def kv_copies(src, dst, sem, a, c, n):
        g = pl.ds(c * n, n)
        return [pltpu.make_async_copy(src.at[a, g, b, :, win], dst.at[a, g, _t(b, 8), :],
                                      sem.at[a, 2 * c + b]) for b in range(2)]

    def k_copy(a, c):
        return kv_copies(k_hbm, kb, k_sem, a, c, CK // 16)

    def v_copy(a, c):
        return kv_copies(v_hbm, vb, v_sem, a, c, CV // 16)

    def start(copies):
        for cp in copies:
            cp.start()

    def wait(copies):
        for cp in copies:
            cp.wait()

    def tile(ref, a, r, cols):
        w = ref[a, _t(r, 8) if isinstance(r, int) else pl.ds(r * 8, 8), :, cols]
        return _bf(w.reshape(64, w.shape[-1]))

    x_copy = pltpu.make_async_copy(x_hbm, x_v, w_sem.at[0])
    wq_copy = pltpu.make_async_copy(wq_hbm, wq_v.bitcast(BF), w_sem.at[1])
    wg_copy = pltpu.make_async_copy(wg_hbm, wg_v.bitcast(BF), w_sem.at[2])
    wu_copy = pltpu.make_async_copy(wu_hbm, wu_v.bitcast(BF), w_sem.at[3])
    wd_copy = pltpu.make_async_copy(wd_hbm, wd_v.bitcast(BF), w_sem.at[4])
    wo_copies = [
        pltpu.make_async_copy(wo_hbm.at[_t(c, H * DH // NWO)],
                              wo_v.bitcast(BF).at[_t(c, H * DH // NWO)], w_sem.at[5 + c])
        for c in range(NWO)]
    x_copy.start()
    wq_copy.start()
    for a in range(2):
        for c in range(NCK):
            start(k_copy(a, c))
    for a in range(2):
        for c in range(NCV):
            start(v_copy(a, c))
    for c in wo_copies:
        c.start()
    wg_copy.start()
    wu_copy.start()
    wd_copy.start()

    def qk(a):
        for r in range(MT):
            part_v[a, r] = _dot(_bf(ql_v[a, :, _t(r)]), tile(k_v, a, r, slice(None)))[_half(r)]
        for j in range(HH - HM):
            qs = [_unpack(qc_v[a, _t(j * RG + g, 8), :]) for g in range(RG)]
            for t in range(NT):
                lo_acc = hi_acc = None
                for g in range(RG):
                    lo, hi = _unpack(k_v[a, (HM + j) * RG + g, :, _t(t)])
                    lo, hi = lo * qs[g][0], hi * qs[g][1]
                    lo_acc = lo if g == 0 else lo_acc + lo
                    hi_acc = hi if g == 0 else hi_acc + hi
                row = HM - 8 + j
                sv_v[a, row:row + 1, _t(t)] = jnp.sum(lo_acc + hi_acc, axis=0, keepdims=True)

    def softmax(a):
        s0 = s1 = None
        for r in range(MT):
            if _half(r).start == 0:
                s0 = part_v[a, r] if s0 is None else s0 + part_v[a, r]
            else:
                s1 = part_v[a, r] if s1 is None else s1 + part_v[a, r]
        rows = lax.broadcasted_iota(jnp.int32, (8, W), 0)
        s = jnp.concatenate([s0, jnp.where(rows < HM - 8, s1, sv_v[a])], axis=0)
        m = jnp.max(s, axis=-1, keepdims=True)
        p = jnp.exp2((s - m) * (DH ** -0.5 * LOG2E))
        rl = 1.0 / jnp.sum(p, axis=-1, keepdims=True)
        pl_v[a] = _pk(p)
        pv_v[a] = p[8:16] * rl[8:16]
        rl_v[a] = jnp.broadcast_to(rl, (16, 128))

    def pv(a):
        rb = 4
        for g0 in range(0, (HH - HM) * RG, rb):
            row = HM - 8 + g0 // RG
            lo_acc, hi_acc = [None] * rb, [None] * rb
            for t in range(NT):
                p = jnp.broadcast_to(pv_v[a, row:row + 1, _t(t)], (8, 128))
                for g in range(rb):
                    lo, hi = _unpack(v_v[a, HM * RG + g0 + g, :, _t(t)])
                    lo, hi = lo * p, hi * p
                    lo_acc[g] = lo if t == 0 else lo_acc[g] + lo
                    hi_acc[g] = hi if t == 0 else hi_acc[g] + hi
            for g in range(rb):
                acc_v[a, 0, _t(g0 + g, 8), :] = lo_acc[g]
                acc_v[a, 1, _t(g0 + g, 8), :] = hi_acc[g]
        for t in range(NT):
            vt = jnp.concatenate([tile(v_v, a, r, _t(t)) for r in range(MT)], axis=1)
            o = _dot(_bf(pl_v[a, :, _t(t)]), vt)
            for r in range(MT):
                part_v[a, r, :, _t(t)] = o[_half(r), _t(r)]

    def o_lhs(a):
        for r in range(MT):
            o = part_v[a, r, :, _t(0)]
            for t in range(1, NT):
                o = o + part_v[a, r, :, _t(t)]
            hs = _half(r)
            col = lax.broadcasted_iota(jnp.int32, (8, 128), 1) + r * 128
            row = lax.broadcasted_iota(jnp.int32, (8, 128), 0) + hs.start
            keep = (col >= row * DH) & (col < (row + 1) * DH)
            o = jnp.where(keep, o * rl_v[a, hs, :], 0.0)
            ol_v[a, :, _t(r)] = _pk(jnp.concatenate([o, jnp.zeros_like(o)], axis=0))

    def out_proj():
        for a in range(2):
            for r in range(MT):
                w = _bf(wo_v[_t(a * HH * PR // 64 + r, 64), :])
                ap_v[a * MT + r] = _dot(_bf(ol_v[a, :, _t(r)]), w)[0:8]
        acc = [None] * (D // 128)
        for a in range(2):
            for g in range((HH - HM) * RG):
                o_lo = jnp.sum(acc_v[a, 0, _t(g, 8), :], axis=-1, keepdims=True)
                o_hi = jnp.sum(acc_v[a, 1, _t(g, 8), :], axis=-1, keepdims=True)
                for c in range(D // 128):
                    lo, hi = _unpack(wo_v[_t((a * HH + HM) * RG + g, 8), _t(c)])
                    y = lo * o_lo + hi * o_hi
                    acc[c] = y if acc[c] is None else acc[c] + y
        ap_v[2 * MT] = jnp.concatenate(acc, axis=1)

    def transpose_v(a):
        def chunk(c, carry):
            wait(v_copy(a, c))

            def tiles(i, carry):
                r = c * (CV // 128) + i
                for t in range(NT):
                    w = pltpu.bitcast(tile(v_v, a, r, _t(t)).T, U32)
                    v_v[a, pl.ds(r * 8, 8), :, _t(t)] = w.reshape(8, 8, 128)
                return carry
            return lax.fori_loop(0, CV // 128, tiles, carry)
        lax.fori_loop(0, HM * DH // CV, chunk, 0)
        for c in range(HM * DH // CV, NCV):
            wait(v_copy(a, c))

    x_copy.wait()
    x0 = jnp.broadcast_to(x_v[...].astype(F32), (8, D))

    def layer(it, x):
        first = it == 0

        def on_first(name, f):
            with scope(name):
                pl.when(first)(f)

        on_first("w_wq", wq_copy.wait)
        xn = _ln(x).astype(BF)
        for a in range(2):
            q = _dot(xn, _bf(wq_v[:, _t(a, HH * DH)]))
            q = jnp.concatenate([q, q], axis=0)
            col = lax.broadcasted_iota(jnp.int32, (16, HM * DH), 1)
            row = lax.broadcasted_iota(jnp.int32, (16, HM * DH), 0)
            keep = (col >= row * DH) & (col < (row + 1) * DH)
            ql_v[a] = _pk(jnp.where(keep, q[:, :HM * DH], 0.0))
            for i in range((HH - HM) * DH // 128):
                qt = q[:, _t(MT + i)].astype(BF)
                qc_v[a, _t(i, 64), :] = pltpu.bitcast(jnp.concatenate([qt] * 8, axis=0).T, U32)

        def wait_k(a):
            for c in range(NCK):
                wait(k_copy(a, c))

        on_first("w_k0", lambda: wait_k(0))
        qk(0)
        on_first("w_k1", lambda: wait_k(1))
        qk(1)
        softmax(0)
        on_first("w_v0", lambda: transpose_v(0))
        pv(0)
        softmax(1)
        on_first("w_v1", lambda: transpose_v(1))
        pv(1)
        o_lhs(0)
        on_first("w_wo0", wo_copies[0].wait)
        o_lhs(1)

        def wait_wo():
            for c in wo_copies[1:]:
                c.wait()
        on_first("w_wo", wait_wo)
        out_proj()

        def wait_gu():
            wg_copy.wait()
            wu_copy.wait()
        on_first("w_gu", wait_gu)
        a = ap_v[0]
        for i in range(1, 2 * MT + 1):
            a = a + ap_v[i]
        x = x + jnp.sum(a, axis=0, keepdims=True)
        xn = _ln(x).astype(BF)
        gate = _dot(xn, _bf(wg_v[...]))
        up = _dot(xn, _bf(wu_v[...]))
        h = (jax.nn.sigmoid(gate) * up).astype(BF)
        on_first("w_wd", wd_copy.wait)
        return x + _dot(h, _bf(wd_v[...]))

    x = lax.fori_loop(0, 2, layer, x0)
    o_ref[...] = x[0:1].astype(o_ref.dtype)


@jax.jit
def pallas_interleave_layers__sliding_block_cached__glu_gated_glu__decode_kernel(
        A_x, A_k_cache, A_v_cache, A_wq, A_wo, B_x, B_w_gate, B_w_up, B_w_down):
    del B_x
    kt = jnp.swapaxes(A_k_cache[0], 1, 2).reshape(2, HH * RG, 2, 8, SK)
    vt = jnp.swapaxes(A_v_cache[0], 1, 2).reshape(2, HH * RG, 2, 8, SK)
    hbm = pl.BlockSpec(memory_space=pl.ANY)
    nv = HH - HM
    out = pl.pallas_call(
        _kernel,
        out_shape=jax.ShapeDtypeStruct((1, D), A_x.dtype),
        in_specs=[hbm] * 8,
        out_specs=pl.BlockSpec(memory_space=pltpu.VMEM),
        scratch_shapes=[
            pltpu.VMEM((1, D), BF),
            pltpu.VMEM((2, HH * RG, 8, W), U32),
            pltpu.VMEM((2, HH * RG, 8, W), U32),
            pltpu.VMEM((D // 2, H * DH), U32),
            pltpu.VMEM((H * PR, D), U32),
            pltpu.VMEM((D // 2, FF), U32),
            pltpu.VMEM((D // 2, FF), U32),
            pltpu.VMEM((FF // 2, D), U32),
            pltpu.VMEM((2, 8, HM * DH), U32),
            pltpu.VMEM((2, nv * PR, 128), U32),
            pltpu.VMEM((2, MT, 8, W), F32),
            pltpu.VMEM((2, 8, W), F32),
            pltpu.VMEM((2, 8, W), U32),
            pltpu.VMEM((2, 8, W), F32),
            pltpu.VMEM((2, 16, 128), F32),
            pltpu.VMEM((2, 2, nv * PR, 128), F32),
            pltpu.VMEM((2, 8, HM * DH), U32),
            pltpu.VMEM((2 * MT + 1, 8, D), F32),
            pltpu.SemaphoreType.DMA((2, 8)),
            pltpu.SemaphoreType.DMA((2, 16)),
            pltpu.SemaphoreType.DMA((9,)),
        ],
        compiler_params=pltpu.CompilerParams(vmem_limit_bytes=127 * 2**20),
        name="interleave_decode",
    )(A_x.reshape(1, D), kt, vt, A_wq, A_wo, B_w_gate, B_w_up, B_w_down)
    return out.reshape(1, 1, D)
```

```python
import jax
import jax.numpy as jnp
import numpy as np
from jax import lax
from jax.experimental import pallas as pl
from jax.experimental.pallas import tpu as pltpu

D, H, DH, SK, FF = 640, 32, 192, 32768, 1536
W = min(4096, max(256, SK // 4))
NT = W // 128
HH = 16
HT = HH * DH // 128
RG = DH // 16
DT, FT = D // 128, FF // 128
KM = (8, 10)
KX = (18, 0)
VM = 10
VT = VM * DH // 128
KE = (3, 4)
KV = tuple(m + 2 * (x > 0) for m, x in zip(KM, KX))
KE0 = (0, KE[0] * (HH - KV[0]), KE[0] * (HH - KV[0]) + KE[1] * (HH - KV[1]))
BF, F32, U32 = jnp.bfloat16, jnp.float32, jnp.uint32
LOG2E = 1.4426950408889634


def _bf(w):
    return pltpu.bitcast(w, BF)


def _unpack(w):
    return (pltpu.bitcast(w << 16, F32),
            pltpu.bitcast(w & np.uint32(0xFFFF0000), F32))


def _dot(a, b):
    return jnp.dot(a, b, preferred_element_type=F32)


def _center(x):
    c = x - jnp.mean(x, axis=-1, keepdims=True)
    return c, lax.rsqrt(jnp.mean(c * c, axis=-1, keepdims=True) + 1e-5)


def _t(i, n=128):
    return slice(i * n, (i + 1) * n)


def _rows16(x):
    return jnp.concatenate([x, x], axis=0)


def _kernel(x_hbm, k_hbm, v_hbm, wq_hbm, wo_hbm, wg_hbm, wu_hbm, wd_hbm, o_ref,
            x_v, k_v, v_v, wq_v, wo_v, wg_v, wu_v, wd_v, ke_v, xl_v,
            ql_v, qc_v, tmp_v, s_v, sx_v, pl_v, pv_v, rl_v, acc_v, ol_v,
            sems):
    win = pl.ds(SK - W, W)
    NWD = 3

    def kv_copies(src, dst, sem):
        return [pltpu.make_async_copy(src.at[:, :, b, :, win], dst.bitcast(BF).at[:, :, _t(b, 8), :],
                                      sems.at[sem]) for b in range(2)]

    def w_copy(src, dst, sem, rows=slice(None)):
        return [pltpu.make_async_copy(src.at[rows], dst.bitcast(BF).at[rows], sems.at[sem])]

    def start(copies):
        for cp in copies:
            cp.start()

    def wait(copies):
        for cp in copies:
            cp.wait()

    def tile(ref, a, r, cols):
        w = ref[a, _t(r, 8) if isinstance(r, int) else pl.ds(r * 8, 8), :, cols]
        return _bf(w.reshape(64, w.shape[-1]))

    xq_copies = [pltpu.make_async_copy(x_hbm, x_v, sems.at[0])] + w_copy(wq_hbm, wq_v, 0)
    v_copies = kv_copies(v_hbm, v_v, 1)
    k_copies = kv_copies(k_hbm, k_v, 2)
    wo_copies = [cp for c in range(2) for cp in w_copy(wo_hbm, wo_v, 3, _t(c, H * DH // 2))]
    gu_copies = w_copy(wg_hbm, wg_v, 0) + w_copy(wu_hbm, wu_v, 0)
    wd_copies = [w_copy(wd_hbm, wd_v, (1, 2, 3)[c], _t(c, FF // NWD)) for c in range(NWD)]
    start(xq_copies + v_copies + k_copies + wo_copies)

    def put_q_row(a, r, q):
        col = lax.broadcasted_iota(jnp.int32, (16, 128), 1) + r * 128
        row = lax.broadcasted_iota(jnp.int32, (16, 128), 0)
        keep = (col >= row * DH) & (col < (row + 1) * DH)
        ql_v[a].bitcast(BF)[:, _t(r)] = jnp.where(keep, _rows16(q), 0.0).astype(BF)

    def put_q_column(a, i, q):
        qt = jnp.concatenate([_rows16(q).astype(BF)] * 8, axis=0).T
        qc_v[a][_t(i, 64), :] = pltpu.bitcast(qt, U32)

    def q_early(c, rs):
        for a in range(2):
            mt = KM[a] * DH // 128
            q = _dot(c, _bf(wq_v[:, (a * HT + mt) * 128:(a + 1) * HT * 128])) * rs
            for i in range(HT - mt):
                put_q_column(a, i, q[:, _t(i)])
                if mt + i < KV[a] * DH // 128:
                    put_q_row(a, mt + i, q[:, _t(i)])
        mt = KM[0] * DH // 128
        q = _dot(c, _bf(wq_v[:, :mt * 128])) * rs
        for r in range(mt):
            put_q_row(0, r, q[:, _t(r)])

    def q_late_mxu():
        n = KM[1] * DH
        for k in range(DT):
            y = _dot(_bf(xl_v[:, _t(k)]), _bf(wq_v[_t(k, 64), HT * 128:HT * 128 + n]))
            tmp_v[0][:, _t(k, n)] = y[0:8]

    def q_late(rs):
        mt = KM[1] * DH // 128
        for r in range(mt):
            q = tmp_v[0][:, _t(r)]
            for k in range(1, DT):
                q = q + tmp_v[0][:, _t(k * mt + r)]
            put_q_row(1, r, q * rs)

    def qk_mxu(a):
        for r in range(KV[a] * DH // 128):
            cols = slice(0, W if r < KM[a] * DH // 128 else KX[a] * 128)
            s = _dot(_bf(ql_v[a][:, _t(r)]), tile(k_v, a, r, cols))
            rows = _t(r // 3, 2)
            if r % 3 == 0:
                s_v[a][rows, cols] = s[rows]
            else:
                sx_v[a][r % 3 - 1, rows, cols] = s[rows]

    def qk_vpu(a):
        for j in range(KM[a], HH):
            qs = [_unpack(qc_v[a][_t((j - KM[a]) * RG + g, 8), :]) for g in range(RG)]
            for t in range(KX[a] if j < KV[a] else 0, NT):
                lo_acc = hi_acc = None
                for g in range(RG):
                    w = k_v[a, j * RG + g, :, _t(t)]
                    if j >= KV[a] and g < KE[a]:
                        lo = ke_v[KE0[a] + (j - KV[a]) * KE[a] + g, :, _t(t)]
                        hi = pltpu.bitcast(w, F32)
                    else:
                        lo, hi = _unpack(w)
                    lo, hi = lo * qs[g][0], hi * qs[g][1]
                    lo_acc = lo if g == 0 else lo_acc + lo
                    hi_acc = hi if g == 0 else hi_acc + hi
                s_v[a][j:j + 1, _t(t)] = jnp.sum(lo_acc + hi_acc, axis=0, keepdims=True)

    def softmax(a):
        m = l = None
        for t in range(NT):
            n = HH if (KV[a] if t < KX[a] else KM[a]) > 8 else 8
            s = s_v[a][0:n, _t(t)] + sx_v[a][0, 0:n, _t(t)] + sx_v[a][1, 0:n, _t(t)]
            s_v[a][0:n, _t(t)] = s
            if n < HH:
                s = jnp.concatenate([s, s_v[a][n:, _t(t)]], axis=0)
            m = s if t == 0 else jnp.maximum(m, s)
        m = jnp.max(m, axis=-1, keepdims=True)
        for t in range(NT):
            p = jnp.exp2((s_v[a][:, _t(t)] - m) * (DH ** -0.5 * LOG2E))
            l = p if t == 0 else l + p
            pv_v[a][:, _t(t)] = p[8:16]
            p0, p1 = p[0:8], p[8:16]
            if t % 4:
                p0, p1 = pltpu.roll(p0, 2 * (t % 4), 0), pltpu.roll(p1, 2 * (t % 4), 0)
            pl_v[a].bitcast(BF)[:, _t(t)] = jnp.concatenate([p0, p1], axis=0).astype(BF)
        rl_v[a][...] = l

    def normalizer(a):
        rl = 1.0 / jnp.sum(rl_v[a][...], axis=-1, keepdims=True)
        rl_v[a][...] = jnp.broadcast_to(rl, (HH, 128))

    def pv_mxu(a):
        tb = 8
        for t0 in range(0, NT, tb):
            for r in range(VT):
                for t in range(t0, t0 + tb):
                    o = _dot(_bf(pl_v[a][:, _t(t)]), tile(v_v, a, r, _t(t)))
                    row = (r // 3 * 2 + 2 * t) % 8
                    src = row + r // 12 * 8
                    tmp_v[a][row:row + 2, _t(r * 8 + t // 4)] = o[src:src + 2]

    def pv_vpu(a):
        rb = 4
        for g0 in range(0, (HH - VM) * RG, rb):
            row = VM + g0 // RG
            lo_acc, hi_acc = [None] * rb, [None] * rb
            for t in range(NT):
                p = jnp.broadcast_to(pv_v[a][row - 8:row - 7, _t(t)], (8, 128))
                for g in range(rb):
                    lo, hi = _unpack(v_v[a, VM * RG + g0 + g, :, _t(t)])
                    lo, hi = lo * p, hi * p
                    lo_acc[g] = lo if t == 0 else lo_acc[g] + lo
                    hi_acc[g] = hi if t == 0 else hi_acc[g] + hi
            for g in range(rb):
                acc_v[a][0, _t(g0 + g, 8), :] = lo_acc[g]
                acc_v[a][1, _t(g0 + g, 8), :] = hi_acc[g]

    def o_lhs(a):
        odd = lax.broadcasted_iota(jnp.int32, (8, 128), 0) % 2 == 1
        low = lax.broadcasted_iota(jnp.int32, (8, 128), 1) < DH - 128
        for r in range(VT):
            o = tmp_v[a][:, _t(r * 8)]
            for i in range(1, NT // 4):
                o = o + tmp_v[a][:, _t(r * 8 + i)]
            h = r // 3 * 2
            rl = jnp.where(odd, jnp.broadcast_to(rl_v[a][h + 1:h + 2, :], (8, 128)),
                           jnp.broadcast_to(rl_v[a][h:h + 1, :], (8, 128)))
            keep = (~odd, odd ^ low, odd)[r % 3]
            o = jnp.where(keep, o * rl, 0.0)
            ol_v[a].bitcast(BF)[:, _t(r)] = jnp.concatenate(
                [o, jnp.zeros_like(o)], axis=0).astype(BF)

    def out_proj_vpu():
        y = None
        for a in range(2):
            for j in range(VM, HH):
                acc = [None] * DT
                for g in range(RG):
                    rows = _t((j - VM) * RG + g, 8)
                    o_lo, o_hi = acc_v[a][0, rows, :], acc_v[a][1, rows, :]
                    if a * (HH - VM) + j - VM >= 0:
                        o_lo = jnp.sum(o_lo, axis=-1, keepdims=True)
                        o_hi = jnp.sum(o_hi, axis=-1, keepdims=True)
                    for c in range(DT):
                        lo, hi = _unpack(wo_v[_t((a * HH + j) * RG + g, 8), _t(c)])
                        z = lo * o_lo + hi * o_hi
                        acc[c] = z if g == 0 else acc[c] + z
                rl = jnp.broadcast_to(rl_v[a][j:j + 1, :], (8, 128))
                z = jnp.concatenate([z * rl for z in acc], axis=1)
                y = z if y is None else y + z
        return y

    def out_proj_mxu():
        for a in range(2):
            for r in range(VT):
                w = _bf(wo_v[_t(a * HT + r, 64), :])
                tmp_v[a][:, _t(r, D)] = _dot(_bf(ol_v[a][:, _t(r)]), w)[0:8]

    def transpose_v(a):
        def tiles(r, carry):
            for t in range(NT):
                w = pltpu.bitcast(tile(v_v, a, r, _t(t)).T, U32)
                v_v[a, pl.ds(r * 8, 8), :, _t(t)] = w.reshape(8, 8, 128)
            return carry
        lax.fori_loop(0, VT, tiles, 0)

    def unpack_k(a):
        def unpack_head(j, carry):
            def unpack_group(g, carry):
                lo, hi = _unpack(k_v[a, (KV[a] + j) * RG + g])
                ke_v[KE0[a] + j * KE[a] + g] = lo
                k_v[a, (KV[a] + j) * RG + g] = pltpu.bitcast(hi, U32)
                return carry
            return lax.fori_loop(0, KE[a], unpack_group, carry)
        if KE[a]:
            lax.fori_loop(0, HH - KV[a], unpack_head, 0)

    for a in range(2):
        sx_v[a][:, 8:16] = jnp.zeros((2, 8, W), F32)
    wait(xq_copies)
    start(gu_copies)
    wait(v_copies)
    start(wd_copies[0])
    for a in range(2):
        transpose_v(a)
    wait(k_copies)
    start(wd_copies[1])
    for a in range(2):
        unpack_k(a)
    x0 = jnp.broadcast_to(x_v[...].astype(F32), (8, D))

    def layer(it, x):
        def on_first(name, f):
            with jax.named_scope(name):
                pl.when(it == 0)(f)
        region = lambda i: pl.when(it * it != i + 2)

        c, rs = _center(x)
        xl_v.bitcast(BF)[...] = _rows16(c).astype(BF)
        q_early(c.astype(BF), rs)

        @region(0)
        def _():
            qk_vpu(0)
            q_late_mxu()
            qk_mxu(0)
        q_late(rs)

        @region(1)
        def _():
            qk_vpu(1)
            softmax(0)
            qk_mxu(1)

        @region(2)
        def _():
            pv_vpu(0)
            normalizer(0)
            softmax(1)
            pv_mxu(0)

        @region(3)
        def _():
            pv_vpu(1)
            normalizer(1)
            o_lhs(0)
            pv_mxu(1)
        for i in range(0):
            a, rows = i // (HH - VM), _t(i % (HH - VM), DH // 2)
            for b in range(2):
                acc_v[a][b, rows, :] = jnp.broadcast_to(
                    jnp.sum(acc_v[a][b, rows, :], axis=-1, keepdims=True), (DH // 2, 128))
        o_lhs(1)
        on_first("w_wo", lambda: (wait(wo_copies), start(sum(wd_copies[2:], [])))[0])

        @region(4)
        def _():
            tmp_v[0][:, _t(VT, D)] = out_proj_vpu()
            out_proj_mxu()
        y = tmp_v[0][:, _t(VT, D)]
        for a in range(2):
            for r in range(VT):
                y = y + tmp_v[a][:, _t(r, D)]
        x = x + jnp.sum(y, axis=0, keepdims=True)

        def glu(arriving):
            c, rs = _center(x)
            c = c.astype(BF)
            if arriving:
                wait(gu_copies)
            hs = []
            for i in range(NWD):
                gate = _dot(c, _bf(wg_v[:, _t(i, FF // NWD)])) * rs
                up = _dot(c, _bf(wu_v[:, _t(i, FF // NWD)])) * rs
                hs.append((jax.nn.sigmoid(gate) * up).astype(BF))
            y = x
            for i in range(NWD):
                if arriving:
                    wait(wd_copies[i])
                y = y + _dot(hs[i], _bf(wd_v[_t(i, FF // NWD // 2), :]))
            return y
        return lax.cond(it == 0, lambda: glu(True), lambda: glu(False))

    x = lax.fori_loop(0, 2, layer, x0)
    o_ref[...] = x[0:1].astype(o_ref.dtype)


@jax.jit
def pallas_interleave_layers__sliding_block_cached__glu_gated_glu__decode_kernel(
        A_x, A_k_cache, A_v_cache, A_wq, A_wo, B_x, B_w_gate, B_w_up, B_w_down):
    del B_x
    kt = jnp.swapaxes(A_k_cache[0], 1, 2).reshape(2, HH * RG, 2, 8, SK)
    vt = jnp.swapaxes(A_v_cache[0], 1, 2).reshape(2, HH * RG, 2, 8, SK)
    hbm = pl.BlockSpec(memory_space=pl.ANY)
    out = pl.pallas_call(
        _kernel,
        out_shape=jax.ShapeDtypeStruct((1, D), A_x.dtype),
        in_specs=[hbm] * 8,
        out_specs=pl.BlockSpec(memory_space=pltpu.VMEM),
        scratch_shapes=[
            pltpu.VMEM((1, D), BF),
            pltpu.VMEM((2, HH * RG, 8, W), U32),
            pltpu.VMEM((2, HH * RG, 8, W), U32),
            pltpu.VMEM((D // 2, H * DH), U32),
            pltpu.VMEM((H * DH // 2, D), U32),
            pltpu.VMEM((D // 2, FF), U32),
            pltpu.VMEM((D // 2, FF), U32),
            pltpu.VMEM((FF // 2, D), U32),
            pltpu.VMEM((max(KE0[2], 1), 8, W), F32),
            pltpu.VMEM((8, D), U32),
            [pltpu.VMEM((8, m * DH), U32) for m in KV],
            [pltpu.VMEM(((HH - m) * DH // 2, 128), U32) for m in KM],
            [pltpu.VMEM((8, 120 * 128), F32)] * 2,
            [pltpu.VMEM((HH, W), F32)] * 2,
            [pltpu.VMEM((2, HH, W), F32)] * 2,
            [pltpu.VMEM((8, W), U32)] * 2,
            [pltpu.VMEM((8, W), F32)] * 2,
            [pltpu.VMEM((HH, 128), F32)] * 2,
            [pltpu.VMEM((2, (HH - VM) * DH // 2, 128), F32)] * 2,
            [pltpu.VMEM((8, VM * DH), U32)] * 2,
            pltpu.SemaphoreType.DMA((4,)),
        ],
        compiler_params=pltpu.CompilerParams(vmem_limit_bytes=128 * 2**20),
        name="interleave_decode",
    )(A_x.reshape(1, D), kt, vt, A_wq, A_wo, B_w_gate, B_w_up, B_w_down)
    return out.reshape(1, 1, D)
```

```python
import jax
import jax.numpy as jnp
import numpy as np
from jax import lax
from jax.experimental import pallas as pl
from jax.experimental.pallas import tpu as pltpu

D, H, DH, SK, FF = 640, 32, 192, 32768, 1536
W = min(4096, max(256, SK // 4))
NT = W // 128
HH = H // 2
HT = HH * DH // 128
RG = DH // 16
DT = D // 128
KM = (8, 10)
KX = (17, 0)
KV = tuple(m + 2 * (x > 0) for m, x in zip(KM, KX))
KE = (4, 3)
KE0 = (0, KE[0] * (HH - KV[0]), KE[0] * (HH - KV[0]) + KE[1] * (HH - KV[1]))
VM = 10
VT = VM * DH // 128
BF, F32, U32 = jnp.bfloat16, jnp.float32, jnp.uint32
LOG2E = 1.4426950408889634


def _bf(w):
    return pltpu.bitcast(w, BF)


def _unpack(w):
    return (pltpu.bitcast(w << 16, F32),
            pltpu.bitcast(w & np.uint32(0xFFFF0000), F32))


def _dot(a, b):
    return jnp.dot(a, b, preferred_element_type=F32)


def _center(x):
    c = x - jnp.mean(x, axis=-1, keepdims=True)
    return c, lax.rsqrt(jnp.mean(c * c, axis=-1, keepdims=True) + 1e-5)


def _t(i, n=128):
    return slice(i * n, (i + 1) * n)


def _rows16(x):
    return jnp.concatenate([x, x], axis=0)


def _kernel(x_hbm, k_hbm, v_hbm, wq_hbm, wo_hbm, wg_hbm, wu_hbm, wd_hbm, o_ref,
            x_v, k_v, v_v, wq_v, wo_v, wg_v, wu_v, wd_v, ke_v, xl_v,
            ql_v, qc_v, tmp_v, s_v, sx_v, pl_v, pv_v, rl_v, acc_v, ol_v, sems):
    wd_rows = (slice(0, 768), slice(768, 1280), slice(1280, FF))

    def kv_copies(src, dst, sem):
        return [pltpu.make_async_copy(src.at[:, :, b, :, pl.ds(SK - W, W)],
                                      dst.bitcast(BF).at[:, :, _t(b, 8), :],
                                      sems.at[sem]) for b in range(2)]

    def w_copy(src, dst, sem, rows=slice(None)):
        return [pltpu.make_async_copy(src.at[rows], dst.bitcast(BF).at[rows], sems.at[sem])]

    def start(copies):
        for cp in copies:
            cp.start()

    def wait(copies):
        for cp in copies:
            cp.wait()

    def tile(ref, a, r, cols):
        w = ref[a, _t(r, 8) if isinstance(r, int) else pl.ds(r * 8, 8), :, cols]
        return _bf(w.reshape(64, w.shape[-1]))

    xq_copies = [pltpu.make_async_copy(x_hbm, x_v, sems.at[0])] + w_copy(wq_hbm, wq_v, 0)
    v_copies = kv_copies(v_hbm, v_v, 1)
    k_copies = kv_copies(k_hbm, k_v, 2)
    wo_copies = [cp for c in range(2) for cp in w_copy(wo_hbm, wo_v, 3, _t(c, H * DH // 2))]
    gu_copies = w_copy(wg_hbm, wg_v, 0) + w_copy(wu_hbm, wu_v, 0)
    wd_copies = [w_copy(wd_hbm, wd_v, 1 + c, rows) for c, rows in enumerate(wd_rows)]

    def put_q_row(a, r, q):
        col = lax.broadcasted_iota(jnp.int32, (16, 128), 1) + r * 128
        row = lax.broadcasted_iota(jnp.int32, (16, 128), 0)
        keep = (col >= row * DH) & (col < (row + 1) * DH)
        ql_v[a].bitcast(BF)[:, _t(r)] = jnp.where(keep, _rows16(q), 0.0).astype(BF)

    def put_q_column(a, i, q):
        qt = jnp.concatenate([_rows16(q).astype(BF)] * 8, axis=0).T
        qc_v[a][_t(i, 64), :] = pltpu.bitcast(qt, U32)

    def q_early(c, rs):
        for a in range(2):
            mt = KM[a] * DH // 128
            q = _dot(c, _bf(wq_v[:, (a * HT + mt) * 128:(a + 1) * HT * 128])) * rs
            for i in range(HT - mt):
                put_q_column(a, i, q[:, _t(i)])
                if mt + i < KV[a] * DH // 128:
                    put_q_row(a, mt + i, q[:, _t(i)])
        mt = KM[0] * DH // 128
        q = _dot(c, _bf(wq_v[:, :mt * 128])) * rs
        for r in range(mt):
            put_q_row(0, r, q[:, _t(r)])

    def q_late_mxu():
        n = KM[1] * DH
        for k in range(DT):
            y = _dot(_bf(xl_v[:, _t(k)]), _bf(wq_v[_t(k, 64), HT * 128:HT * 128 + n]))
            tmp_v[0][:, _t(k, n)] = y[0:8]

    def q_late(rs):
        mt = KM[1] * DH // 128
        for r in range(mt):
            q = tmp_v[0][:, _t(r)]
            for k in range(1, DT):
                q = q + tmp_v[0][:, _t(k * mt + r)]
            put_q_row(1, r, q * rs)

    def qk_mxu(a):
        for r in range(KV[a] * DH // 128):
            cols = slice(0, W if r < KM[a] * DH // 128 else KX[a] * 128)
            s = _dot(_bf(ql_v[a][:, _t(r)]), tile(k_v, a, r, cols))
            rows = _t(r // 3, 2)
            if r % 3 == 0:
                s_v[a][rows, cols] = s[rows]
            else:
                sx_v[a][r % 3 - 1, rows, cols] = s[rows]

    def qk_vpu(a):
        for j in range(KM[a], HH):
            qs = [_unpack(qc_v[a][_t((j - KM[a]) * RG + g, 8), :]) for g in range(RG)]
            for t in range(KX[a] if j < KV[a] else 0, NT):
                for g in range(RG):
                    w = k_v[a, j * RG + g, :, _t(t)]
                    if j >= KV[a] and g < KE[a]:
                        lo = ke_v[KE0[a] + (j - KV[a]) * KE[a] + g, :, _t(t)]
                        hi = pltpu.bitcast(w, F32)
                    else:
                        lo, hi = _unpack(w)
                    y = lo * qs[g][0] + hi * qs[g][1]
                    s = y if g == 0 else s + y
                s_v[a][j:j + 1, _t(t)] = jnp.sum(s, axis=0, keepdims=True)

    def softmax(a):
        for t in range(NT):
            n = HH if (KV[a] if t < KX[a] else KM[a]) > 8 else 8
            s = s_v[a][0:n, _t(t)] + sx_v[a][0, 0:n, _t(t)] + sx_v[a][1, 0:n, _t(t)]
            s_v[a][0:n, _t(t)] = s
            if n < HH:
                s = jnp.concatenate([s, s_v[a][n:, _t(t)]], axis=0)
            m = s if t == 0 else jnp.maximum(m, s)
        m = jnp.max(m, axis=-1, keepdims=True)
        for t in range(NT):
            p = jnp.exp2((s_v[a][:, _t(t)] - m) * (DH ** -0.5 * LOG2E))
            l = p if t == 0 else l + p
            pv_v[a][:, _t(t)] = p[8:16]
            p0, p1 = p[0:8], p[8:16]
            if t % 4:
                p0, p1 = pltpu.roll(p0, 2 * (t % 4), 0), pltpu.roll(p1, 2 * (t % 4), 0)
            pl_v[a].bitcast(BF)[:, _t(t)] = jnp.concatenate([p0, p1], axis=0).astype(BF)
        rl_v[a][...] = l

    def normalizer(a):
        rl = 1.0 / jnp.sum(rl_v[a][...], axis=-1, keepdims=True)
        rl_v[a][...] = jnp.broadcast_to(rl, (HH, 128))

    def pv_mxu(a):
        tb = 8
        for t0 in range(0, NT, tb):
            for r in range(VT):
                for t in range(t0, t0 + tb):
                    o = _dot(_bf(pl_v[a][:, _t(t)]), tile(v_v, a, r, _t(t)))
                    row = (r // 3 * 2 + 2 * t) % 8
                    src = row + r // 12 * 8
                    tmp_v[a][row:row + 2, _t(r * 8 + t // 4)] = o[src:src + 2]

    def pv_vpu(a):
        rb = 4
        for g0 in range(0, (HH - VM) * RG, rb):
            row = VM + g0 // RG
            lo_acc, hi_acc = [None] * rb, [None] * rb
            for t in range(NT):
                p = jnp.broadcast_to(pv_v[a][row - 8:row - 7, _t(t)], (8, 128))
                for g in range(rb):
                    lo, hi = _unpack(v_v[a, VM * RG + g0 + g, :, _t(t)])
                    lo, hi = lo * p, hi * p
                    lo_acc[g] = lo if t == 0 else lo_acc[g] + lo
                    hi_acc[g] = hi if t == 0 else hi_acc[g] + hi
            for g in range(rb):
                acc_v[a][0, _t(g0 + g, 8), :] = lo_acc[g]
                acc_v[a][1, _t(g0 + g, 8), :] = hi_acc[g]

    def o_lhs(a):
        odd = lax.broadcasted_iota(jnp.int32, (8, 128), 0) % 2 == 1
        low = lax.broadcasted_iota(jnp.int32, (8, 128), 1) < DH - 128
        for r in range(VT):
            o = tmp_v[a][:, _t(r * 8)]
            for i in range(1, NT // 4):
                o = o + tmp_v[a][:, _t(r * 8 + i)]
            h = r // 3 * 2
            rl = jnp.where(odd, jnp.broadcast_to(rl_v[a][h + 1:h + 2, :], (8, 128)),
                           jnp.broadcast_to(rl_v[a][h:h + 1, :], (8, 128)))
            keep = (~odd, odd ^ low, odd)[r % 3]
            o = jnp.where(keep, o * rl, 0.0)
            ol_v[a].bitcast(BF)[:, _t(r)] = jnp.concatenate(
                [o, jnp.zeros_like(o)], axis=0).astype(BF)

    def out_proj_vpu():
        y = None
        for a in range(2):
            for j in range(VM, HH):
                acc = [None] * DT
                for g in range(RG):
                    rows = _t((j - VM) * RG + g, 8)
                    o_lo = jnp.sum(acc_v[a][0, rows, :], axis=-1, keepdims=True)
                    o_hi = jnp.sum(acc_v[a][1, rows, :], axis=-1, keepdims=True)
                    for c in range(DT):
                        lo, hi = _unpack(wo_v[_t((a * HH + j) * RG + g, 8), _t(c)])
                        z = lo * o_lo + hi * o_hi
                        acc[c] = z if g == 0 else acc[c] + z
                rl = jnp.broadcast_to(rl_v[a][j:j + 1, :], (8, 128))
                z = jnp.concatenate([z * rl for z in acc], axis=1)
                y = z if y is None else y + z
        return y

    def out_proj_mxu():
        for a in range(2):
            for r in range(VT):
                w = _bf(wo_v[_t(a * HT + r, 64), :])
                tmp_v[a][:, _t(r, D)] = _dot(_bf(ol_v[a][:, _t(r)]), w)[0:8]

    def transpose_v(a):
        def tiles(r, carry):
            for t in range(NT):
                w = pltpu.bitcast(tile(v_v, a, r, _t(t)).T, U32)
                v_v[a, pl.ds(r * 8, 8), :, _t(t)] = w.reshape(8, 8, 128)
            return carry
        lax.fori_loop(0, VT, tiles, 0)

    def unpack_k(a):
        def unpack_head(j, carry):
            def unpack_group(g, carry):
                lo, hi = _unpack(k_v[a, (KV[a] + j) * RG + g])
                ke_v[KE0[a] + j * KE[a] + g] = lo
                k_v[a, (KV[a] + j) * RG + g] = pltpu.bitcast(hi, U32)
                return carry
            return lax.fori_loop(0, KE[a], unpack_group, carry)
        lax.fori_loop(0, HH - KV[a], unpack_head, 0)

    start(xq_copies + v_copies + k_copies + wo_copies)
    for a in range(2):
        sx_v[a][:, 8:16] = jnp.zeros((2, 8, W), F32)
    wait(xq_copies)
    start(gu_copies)
    wait(v_copies)
    start(wd_copies[0])
    for a in range(2):
        transpose_v(a)
    wait(k_copies)
    start(wd_copies[1])
    for a in range(2):
        unpack_k(a)

    def layer(it, x):
        def region(i):
            return pl.when(it * it != i + 2)

        c, rs = _center(x)
        xl_v.bitcast(BF)[...] = _rows16(c).astype(BF)
        q_early(c.astype(BF), rs)

        @region(0)
        def _():
            qk_vpu(0)
            q_late_mxu()
            qk_mxu(0)
        q_late(rs)

        @region(1)
        def _():
            qk_vpu(1)
            softmax(0)
            qk_mxu(1)

        @region(2)
        def _():
            pv_vpu(0)
            normalizer(0)
            softmax(1)
            pv_mxu(0)

        @region(3)
        def _():
            pv_vpu(1)
            normalizer(1)
            o_lhs(0)
            pv_mxu(1)
        o_lhs(1)

        @pl.when(it == 0)
        def _():
            wait(wo_copies)
            start(wd_copies[2])

        @region(4)
        def _():
            tmp_v[0][:, _t(VT, D)] = out_proj_vpu()
            out_proj_mxu()
        y = tmp_v[0][:, _t(VT, D)]
        for a in range(2):
            for r in range(VT):
                y = y + tmp_v[a][:, _t(r, D)]
        x = x + jnp.sum(y, axis=0, keepdims=True)

        def glu(arriving):
            c, rs = _center(x)
            c = c.astype(BF)
            if arriving:
                wait(gu_copies)
            hs = []
            for i in range(3):
                gate = _dot(c, _bf(wg_v[:, _t(i, FF // 3)])) * rs
                up = _dot(c, _bf(wu_v[:, _t(i, FF // 3)])) * rs
                hs.append((jax.nn.sigmoid(gate) * up).astype(BF))
            h = jnp.concatenate(hs, axis=1)
            y = x
            for rows, copies in zip(wd_rows, wd_copies):
                if arriving:
                    wait(copies)
                y = y + _dot(h[:, rows], _bf(wd_v[rows.start // 2:rows.stop // 2, :]))
            return y
        return lax.cond(it == 0, lambda: glu(True), lambda: glu(False))

    x = lax.fori_loop(0, 2, layer, jnp.broadcast_to(x_v[...].astype(F32), (8, D)))
    o_ref[...] = x[0:1].astype(o_ref.dtype)


@jax.jit
def pallas_interleave_layers__sliding_block_cached__glu_gated_glu__decode_kernel(
        A_x, A_k_cache, A_v_cache, A_wq, A_wo, B_x, B_w_gate, B_w_up, B_w_down):
    del B_x
    kt = jnp.swapaxes(A_k_cache[0], 1, 2).reshape(2, HH * RG, 2, 8, SK)
    vt = jnp.swapaxes(A_v_cache[0], 1, 2).reshape(2, HH * RG, 2, 8, SK)
    out = pl.pallas_call(
        _kernel,
        out_shape=jax.ShapeDtypeStruct((1, D), A_x.dtype),
        in_specs=[pl.BlockSpec(memory_space=pl.ANY)] * 8,
        out_specs=pl.BlockSpec(memory_space=pltpu.VMEM),
        scratch_shapes=[
            pltpu.VMEM((1, D), BF),
            pltpu.VMEM((2, HH * RG, 8, W), U32),
            pltpu.VMEM((2, HH * RG, 8, W), U32),
            pltpu.VMEM((D // 2, H * DH), U32),
            pltpu.VMEM((H * DH // 2, D), U32),
            pltpu.VMEM((D // 2, FF), U32),
            pltpu.VMEM((D // 2, FF), U32),
            pltpu.VMEM((FF // 2, D), U32),
            pltpu.VMEM((KE0[2], 8, W), F32),
            pltpu.VMEM((8, D), U32),
            [pltpu.VMEM((8, m * DH), U32) for m in KV],
            [pltpu.VMEM(((HH - m) * DH // 2, 128), U32) for m in KM],
            [pltpu.VMEM((8, VT * NT // 4 * 128), F32)] * 2,
            [pltpu.VMEM((HH, W), F32)] * 2,
            [pltpu.VMEM((2, HH, W), F32)] * 2,
            [pltpu.VMEM((8, W), U32)] * 2,
            [pltpu.VMEM((8, W), F32)] * 2,
            [pltpu.VMEM((HH, 128), F32)] * 2,
            [pltpu.VMEM((2, (HH - VM) * DH // 2, 128), F32)] * 2,
            [pltpu.VMEM((8, VM * DH), U32)] * 2,
            pltpu.SemaphoreType.DMA((4,)),
        ],
        compiler_params=pltpu.CompilerParams(vmem_limit_bytes=128 * 2**20),
        name="interleave_decode",
    )(A_x.reshape(1, D), kt, vt, A_wq, A_wo, B_w_gate, B_w_up, B_w_down)
    return out.reshape(1, 1, D)
```
